```python
import jax
import jax.numpy as jnp

def _softmax(x, axis=-1):
    return jax.nn.softmax(x, axis=axis)

def _gelu(x):
    return jax.nn.gelu(x, approximate=True)

def _silu(x):
    return jax.nn.silu(x)

def _sigmoid(x):
    return jax.nn.sigmoid(x)

def _layernorm(x, axis=-1, eps=1e-05):
    m = jnp.mean(x, axis=axis, keepdims=True)
    v = jnp.var(x, axis=axis, keepdims=True)
    return (x - m) / jnp.sqrt(v + eps)

def _scatter_add(tgt, idx, src, axis=0):
    return tgt.at[idx].add(src)

def _segment_sum(src, seg, n):
    return jax.ops.segment_sum(src, seg, n)

class _Rng:

    def __init__(self, key):
        self._k = key

    def _next(self):
        self._k, sub = jax.random.split(self._k)
        return sub

    def normal(self, shape):
        return jax.random.normal(self._next(), shape, dtype=jnp.bfloat16)

    def randint(self, lo, hi, shape):
        return jax.random.randint(self._next(), shape, lo, hi, dtype=jnp.int32)

    def uniform(self, shape, lo=0.0, hi=1.0):
        return jax.random.uniform(self._next(), shape, jnp.bfloat16, lo, hi)

    def permutation(self, n):
        return jax.random.permutation(self._next(), n)
kernel_name = 'adaLN_cond__gqa_block_cached__moe_arch_mod__decode'

def setup_inputs():
    _rng = _Rng(jax.random.key(int.from_bytes(__import__("os").urandom(4), "little")))
    _w = lambda a: (lambda t: t.astype(jnp.bfloat16) if jnp.issubdtype(t.dtype, jnp.floating) else t)(jnp.asarray(a))

    def _A_setup():
        B, Sq, D = (4, 1, 512)
        Hq, Hkv, Sk, Dh = (32, 32, 8192, 128)
        assert Hq % Hkv == 0, (Hq, Hkv)
        return {'x': _w((lambda *s: _rng.normal(s) * 0.05)(B, Sq, D)), 'k_cache': _w((lambda *s: _rng.normal(s) * 0.05)(B, Hkv, Sk, Dh)), 'v_cache': _w((lambda *s: _rng.normal(s) * 0.05)(B, Hkv, Sk, Dh)), 'wq': _w((lambda *s: _rng.normal(s) * 0.05)(D, Hq * Dh) * D ** (-0.5)), 'wo': _w((lambda *s: _rng.normal(s) * 0.05)(Hq * Dh, D) * (Hq * Dh) ** (-0.5))}
    _A_in = _A_setup()

    def _B_setup():
        B, S, D, F, C = (4, 1, 512, 1376, 1)
        return {'x': _w((lambda *s: _rng.normal(s) * 0.05)(B, S, D)), 'w_r': _w((lambda *s: _rng.normal(s) * 0.05)(D)), 'w_gate': _w((lambda *s: _rng.normal(s) * 0.05)(D, F)), 'w_up': _w((lambda *s: _rng.normal(s) * 0.05)(D, F)), 'w_down': _w((lambda *s: _rng.normal(s) * 0.05)(F, D))}
    _B_in = _B_setup()
    return {'A_x': _A_in['x'], 'A_k_cache': _A_in['k_cache'], 'A_v_cache': _A_in['v_cache'], 'A_wq': _A_in['wq'], 'A_wo': _A_in['wo'], 'B_x': _B_in['x'], 'B_w_r': _B_in['w_r'], 'B_w_gate': _B_in['w_gate'], 'B_w_up': _B_in['w_up'], 'B_w_down': _B_in['w_down'], 'c': _w((lambda *s: _rng.normal(s) * 0.05)(4, 512)), 'w_mod': _w((lambda *s: _rng.normal(s) * 0.05)(512, 6 * 512) * 512 ** (-0.5))}

def reference(A_x, A_k_cache, A_v_cache, A_wq, A_wo, B_x, B_w_r, B_w_gate, B_w_up, B_w_down, c, w_mod):

    def _A_ref(x, k_cache, v_cache, wq, wo):
        B, Sq, D = x.shape
        Hq, Dh = (32, 128)
        Hkv = k_cache.shape[1]
        rep = Hq // Hkv
        q = (lambda x, *d: x.transpose(*d))((x @ wq).reshape(B, Sq, Hq, Dh), 0, 2, 1, 3)
        k = jnp.repeat(k_cache, rep, axis=1)
        v = jnp.repeat(v_cache, rep, axis=1)
        scores = jnp.einsum('bhqd,bhkd->bhqk', q, k) * Dh ** (-0.5)
        p = _softmax(scores, axis=-1)
        o = jnp.einsum('bhqk,bhkd->bhqd', p, v)
        return (lambda x, *d: x.transpose(*d))(o, 0, 2, 1, 3).reshape(B, Sq, Hq * Dh) @ wo

    def _B_ref(x, w_r, w_gate, w_up, w_down):
        B, S, D = x.shape
        C = 1
        r = x @ w_r
        idx = jnp.argsort(-r, axis=-1)[:, :C]
        idx_e = jnp.repeat(idx.reshape(B, C, 1), D, axis=2)
        x_sel = jnp.take_along_axis(x, idx_e, axis=1)
        g = _silu(x_sel @ w_gate)
        u = x_sel @ w_up
        y = g * u @ w_down
        r_sel = _sigmoid(jnp.take_along_axis(r, idx, axis=1))
        y = y * r_sel.reshape(B, C, 1)
        b_off = (jnp.arange(B) * S).reshape(B, 1)
        flat_idx = (idx + b_off).reshape(B * C)
        zero = (x * 0.0).reshape(B * S, D)
        upd = _scatter_add(zero, flat_idx, y.reshape(B * C, D), axis=0)
        return x + upd.reshape(B, S, D)
    x = A_x
    mod = (_silu(c) @ w_mod).reshape(c.shape[0], 6, 1, -1)
    sa, ca, ga, sb, cb, gb = (mod[:, 0].copy(), mod[:, 1].copy(), mod[:, 2].copy(), mod[:, 3].copy(), mod[:, 4].copy(), mod[:, 5].copy())
    h = _layernorm(x, axis=-1) * (1 + ca) + sa
    x = x + ga * _A_ref(h, A_k_cache, A_v_cache, A_wq, A_wo)
    h = _layernorm(x, axis=-1) * (1 + cb) + sb
    x = x + gb * _B_ref(h, B_w_r, B_w_gate, B_w_up, B_w_down)
    return x
```

```python
import functools

import jax
import jax.numpy as jnp
from jax import lax
import jax.experimental.pallas as pl
import jax.experimental.pallas.tpu as pltpu

NT = (((1,), (1,)), ((), ()))
NB = 4


def _layernorm(x, eps=1e-5):
    m = jnp.mean(x, axis=-1, keepdims=True)
    d = x - m
    v = jnp.mean(d * d, axis=-1, keepdims=True)
    return d / jnp.sqrt(v + eps)


def _kernel(x_hbm, k_hbm, v_hbm, wq_hbm, wo_hbm, wr_hbm, wg_hbm, wu_hbm, wd_hbm,
            c_hbm, wmod_hbm, out_ref,
            kbuf, vbuf, x_vm, c_vm, wmod_vm, wq_vm, wo_vm, wr_vm, wg_vm, wu_vm, wd_vm,
            q_scr, o_scr, ksem, vsem, wsem, *, B, H, Dh, D):
    f32, bf16 = jnp.float32, jnp.bfloat16
    N = B * H

    def wcopy(src, dst, i):
        return pltpu.make_async_copy(src, dst, wsem.at[i])

    cp_c = wcopy(c_hbm, c_vm, 0)
    cp_x = wcopy(x_hbm, x_vm, 1)
    cp_wmod = wcopy(wmod_hbm, wmod_vm, 2)
    cp_wq = wcopy(wq_hbm, wq_vm, 3)
    cp_wo = wcopy(wo_hbm, wo_vm, 4)
    cp_wr = wcopy(wr_hbm, wr_vm, 5)
    cp_wg = wcopy(wg_hbm, wg_vm, 6)
    cp_wu = wcopy(wu_hbm, wu_vm, 7)
    cp_wd = wcopy(wd_hbm, wd_vm, 8)

    def kcopy(i, slot):
        return pltpu.make_async_copy(k_hbm.at[i // H, i % H], kbuf.at[slot], ksem.at[slot])

    def vcopy(i, slot):
        return pltpu.make_async_copy(v_hbm.at[i // H, i % H], vbuf.at[slot], vsem.at[slot])

    cp_c.start()
    cp_x.start()
    cp_wmod.start()
    cp_wq.start()
    for j in range(NB):
        kcopy(j, j).start()
        vcopy(j, j).start()

    cp_c.wait()
    cp_wmod.wait()
    c = c_vm[...].astype(f32)
    sc = (c * jax.nn.sigmoid(c)).astype(bf16)
    mod = jnp.dot(sc, wmod_vm[...], preferred_element_type=f32)
    sa, ca, ga, sb, cb, gb = (mod[:, i * D:(i + 1) * D] for i in range(6))
    cp_x.wait()
    x = x_vm[...].astype(f32)
    h = (_layernorm(x) * (1.0 + ca) + sa).astype(bf16)
    cp_wq.wait()
    q = jnp.dot(h, wq_vm[...], preferred_element_type=f32)
    for hh in range(H):
        q_scr[hh] = q[:, hh * Dh:(hh + 1) * Dh]
        o_scr[hh] = jnp.zeros((B, Dh), f32)

    scale = float(Dh) ** -0.5
    row = lax.broadcasted_iota(jnp.int32, (B, Dh), 0)

    def body(i, carry):
        slot = i % NB
        b = i // H
        hd = i % H
        kcopy(i, slot).wait()
        qh = q_scr[hd].astype(bf16)
        s = lax.dot_general(qh, kbuf[slot], NT, preferred_element_type=f32)

        @pl.when(i + NB < N)
        def _():
            kcopy(i + NB, slot).start()

        s = s * scale
        m = jnp.max(s, axis=-1, keepdims=True)
        p = jnp.exp(s - m)
        l = jnp.sum(p, axis=-1, keepdims=True)
        vcopy(i, slot).wait()
        o = jnp.dot(p.astype(bf16), vbuf[slot], preferred_element_type=f32)

        @pl.when(i + NB < N)
        def _():
            vcopy(i + NB, slot).start()

        @pl.when(i + NB == N)
        def _():
            cp_wo.start()
            cp_wr.start()
            cp_wg.start()
            cp_wu.start()
            cp_wd.start()

        o_scr[hd] = jnp.where(row == b, o / l, o_scr[hd])
        return carry

    lax.fori_loop(0, N, body, 0)

    cp_wo.wait()
    o_all = jnp.concatenate([o_scr[hh] for hh in range(H)], axis=1).astype(bf16)
    attn = jnp.dot(o_all, wo_vm[...], preferred_element_type=f32)
    x2 = x + ga * attn
    h2 = _layernorm(x2) * (1.0 + cb) + sb
    h2b = h2.astype(bf16)
    cp_wr.wait()
    r = jnp.sum(h2 * wr_vm[...].astype(f32).reshape(1, D), axis=-1, keepdims=True)
    cp_wg.wait()
    g = lax.dot_general(h2b, wg_vm[...], NT, preferred_element_type=f32)
    g = g * jax.nn.sigmoid(g)
    cp_wu.wait()
    u = lax.dot_general(h2b, wu_vm[...], NT, preferred_element_type=f32)
    gu = (g * u).astype(bf16)
    cp_wd.wait()
    y = jnp.dot(gu, wd_vm[...], preferred_element_type=f32)
    y = y * jax.nn.sigmoid(r)
    upd = h2 * 0.0 + y
    out = x2 + gb * (h2 + upd)
    out_ref[...] = out.astype(out_ref.dtype)


@jax.jit
def pallas_adaLN_cond__gqa_block_cached__moe_arch_mod__decode_kernel(
    A_x: jax.Array,
    A_k_cache: jax.Array,
    A_v_cache: jax.Array,
    A_wq: jax.Array,
    A_wo: jax.Array,
    B_x: jax.Array,
    B_w_r: jax.Array,
    B_w_gate: jax.Array,
    B_w_up: jax.Array,
    B_w_down: jax.Array,
    c: jax.Array,
    w_mod: jax.Array,
):
    del B_x
    B, Sq, D = A_x.shape
    _, H, S, Dh = A_k_cache.shape
    assert Sq == 1 and A_wq.shape == (D, H * Dh)

    x2d = A_x.reshape(B, D)
    wg_t = B_w_gate.T
    wu_t = B_w_up.T

    def vm(a):
        return pltpu.VMEM(a.shape, a.dtype)

    any_spec = pl.BlockSpec(memory_space=pltpu.HBM)
    return pl.pallas_call(
        functools.partial(_kernel, B=B, H=H, Dh=Dh, D=D),
        out_shape=jax.ShapeDtypeStruct((B, D), A_x.dtype),
        in_specs=[any_spec] * 11,
        out_specs=pl.BlockSpec(memory_space=pltpu.VMEM),
        scratch_shapes=[
            pltpu.VMEM((NB, S, Dh), A_k_cache.dtype),
            pltpu.VMEM((NB, S, Dh), A_v_cache.dtype),
            vm(x2d), vm(c), vm(w_mod), vm(A_wq), vm(A_wo), vm(B_w_r),
            vm(wg_t), vm(wu_t), vm(B_w_down),
            pltpu.VMEM((H, B, Dh), jnp.float32),
            pltpu.VMEM((H, B, Dh), jnp.float32),
            pltpu.SemaphoreType.DMA((NB,)),
            pltpu.SemaphoreType.DMA((NB,)),
            pltpu.SemaphoreType.DMA((9,)),
        ],
        compiler_params=pltpu.CompilerParams(
            vmem_limit_bytes=100 * 1024 * 1024,
        ),
    )(x2d, A_k_cache, A_v_cache, A_wq, A_wo, B_w_r, wg_t, wu_t, B_w_down, c, w_mod).reshape(B, Sq, D)
```

```python
import functools

import jax
import jax.numpy as jnp
from jax import lax
import jax.experimental.pallas as pl
import jax.experimental.pallas.tpu as pltpu

NT = (((1,), (1,)), ((), ()))
G = 8
C = 512
P = 128
NB = 3
DBC = False


def _layernorm(x, eps=1e-5):
    m = jnp.mean(x, axis=-1, keepdims=True)
    d = x - m
    v = jnp.mean(d * d, axis=-1, keepdims=True)
    return d / jnp.sqrt(v + eps)


def _kernel(x_hbm, k_hbm, v_hbm, wq_hbm, wo_hbm, wr_hbm, wg_hbm, wu_hbm, wd_hbm,
            c_hbm, wmod_hbm, out_ref,
            kbuf, vbuf, x_vm, c_vm, wmod_vm, wq_vm, wo_vm, wr_vm, wg_vm, wu_vm, wd_vm,
            q_scr, o_scr, ksem, vsem, wsem, *, B, H, S, Dh, D):
    f32, bf16 = jnp.float32, jnp.bfloat16
    NG = B * H // G
    NC = S // C
    N = NG * NC

    def wcopy(src, dst, i):
        return pltpu.make_async_copy(src, dst, wsem.at[i])

    cp_c = wcopy(c_hbm, c_vm, 0)
    cp_x = wcopy(x_hbm, x_vm, 1)
    cp_wmod = wcopy(wmod_hbm, wmod_vm, 2)
    cp_wq = wcopy(wq_hbm, wq_vm, 3)
    cp_wo = wcopy(wo_hbm, wo_vm, 4)
    cp_wr = wcopy(wr_hbm, wr_vm, 5)
    cp_wg = wcopy(wg_hbm, wg_vm, 6)
    cp_wu = wcopy(wu_hbm, wu_vm, 7)
    cp_wd = wcopy(wd_hbm, wd_vm, 8)

    def start_step(i, slot):
        grp = i // NC
        c = i % NC
        b = grp // (H // G)
        h0 = (grp % (H // G)) * G
        for j in range(C // P):
            for g in range(G):
                src = (b, h0 + g, pl.ds(c * C + j * P, P))
                dst = (slot, g, pl.ds(j * P, P))
                pltpu.make_async_copy(k_hbm.at[src], kbuf.at[dst], ksem.at[slot]).start(priority=0)
                pltpu.make_async_copy(v_hbm.at[src], vbuf.at[dst], vsem.at[slot]).start(priority=1)

    def wait_k(slot):
        pltpu.make_async_copy(kbuf.at[slot], kbuf.at[slot], ksem.at[slot]).wait()

    def wait_v(slot):
        pltpu.make_async_copy(vbuf.at[slot], vbuf.at[slot], vsem.at[slot]).wait()

    cp_c.start()
    cp_x.start()
    cp_wmod.start()
    cp_wq.start()
    for j in range(NB - 1):
        start_step(j, j)

    cp_c.wait()
    cp_wmod.wait()
    c = c_vm[...].astype(f32)
    sc = (c * jax.nn.sigmoid(c)).astype(bf16)
    mod = jnp.dot(sc, wmod_vm[...], preferred_element_type=f32)
    sa, ca, ga, sb, cb, gb = (mod[:, i * D:(i + 1) * D] for i in range(6))
    cp_x.wait()
    x = x_vm[...].astype(f32)
    h = (_layernorm(x) * (1.0 + ca) + sa).astype(bf16)
    cp_wq.wait()
    q = jnp.dot(h, wq_vm[...], preferred_element_type=f32)
    for hh in range(H):
        q_scr[pl.ds(hh, B, stride=H), :] = q[:, hh * Dh:(hh + 1) * Dh]

    scale = float(Dh) ** -0.5
    row = lax.broadcasted_iota(jnp.int32, (G, Dh), 0)

    def group(grp, carry):
        qg = q_scr[pl.ds(pl.multiple_of(grp * G, G), G), :].astype(bf16)

        def step(c, carry):
            m_prev, l_prev, o_prev = carry
            i = grp * NC + c
            slot = i % NB

            @pl.when(i + NB - 1 < N)
            def _():
                start_step(i + NB - 1, (i + NB - 1) % NB)

            @pl.when(i + NB - 1 == N)
            def _():
                cp_wo.start()
                cp_wr.start()
                cp_wg.start()
                cp_wu.start()
                cp_wd.start()

            wait_k(slot)
            s = None
            for g in range(G):
                sg = lax.dot_general(qg, kbuf[slot, g], NT, preferred_element_type=f32)
                s = sg if s is None else jnp.where(row[:, :1] == g, sg, s)
            s = s * scale
            m_new = jnp.maximum(m_prev, jnp.max(s, axis=-1, keepdims=True))
            m_safe = jnp.where(m_new == -jnp.inf, 0.0, m_new)
            p = jnp.exp(s - m_safe)
            alpha = jnp.exp(m_prev - m_safe)
            l_new = alpha * l_prev + jnp.sum(p, axis=-1, keepdims=True)
            pb = p.astype(bf16)
            wait_v(slot)
            r = None
            for g in range(G):
                rg = jnp.dot(pb, vbuf[slot, g], preferred_element_type=f32)
                r = rg if r is None else jnp.where(row == g, rg, r)
            o_new = alpha * o_prev + r
            return m_new, l_new, o_new

        init = (jnp.full((G, 1), -jnp.inf, f32), jnp.zeros((G, 1), f32), jnp.zeros((G, Dh), f32))
        m, l, o = lax.fori_loop(0, NC, step, init)
        o_scr[pl.ds(pl.multiple_of(grp * G, G), G), :] = o / l
        return carry

    lax.fori_loop(0, NG, group, 0)

    o_all = jnp.concatenate(
        [o_scr[pl.ds(hh, B, stride=H), :] for hh in range(H)], axis=1).astype(bf16)
    cp_wo.wait()
    attn = jnp.dot(o_all, wo_vm[...], preferred_element_type=f32)
    x2 = x + ga * attn
    h2 = _layernorm(x2) * (1.0 + cb) + sb
    h2b = h2.astype(bf16)
    cp_wr.wait()
    r = jnp.sum(h2 * wr_vm[...].astype(f32).reshape(1, D), axis=-1, keepdims=True)
    cp_wg.wait()
    g = lax.dot_general(h2b, wg_vm[...], NT, preferred_element_type=f32)
    g = g * jax.nn.sigmoid(g)
    cp_wu.wait()
    u = lax.dot_general(h2b, wu_vm[...], NT, preferred_element_type=f32)
    gu = (g * u).astype(bf16)
    cp_wd.wait()
    y = jnp.dot(gu, wd_vm[...], preferred_element_type=f32)
    y = y * jax.nn.sigmoid(r)
    upd = h2 * 0.0 + y
    out = x2 + gb * (h2 + upd)
    out_ref[...] = out.astype(out_ref.dtype)


@jax.jit
def pallas_adaLN_cond__gqa_block_cached__moe_arch_mod__decode_kernel(
    A_x: jax.Array,
    A_k_cache: jax.Array,
    A_v_cache: jax.Array,
    A_wq: jax.Array,
    A_wo: jax.Array,
    B_x: jax.Array,
    B_w_r: jax.Array,
    B_w_gate: jax.Array,
    B_w_up: jax.Array,
    B_w_down: jax.Array,
    c: jax.Array,
    w_mod: jax.Array,
):
    del B_x
    B, Sq, D = A_x.shape
    _, H, S, Dh = A_k_cache.shape
    assert Sq == 1 and A_wq.shape == (D, H * Dh)
    assert H % G == 0 and S % C == 0 and C % P == 0

    x2d = A_x.reshape(B, D)
    wg_t = B_w_gate.T
    wu_t = B_w_up.T

    def vm(a):
        return pltpu.VMEM(a.shape, a.dtype)

    any_spec = pl.BlockSpec(memory_space=pltpu.HBM)
    return pl.pallas_call(
        functools.partial(_kernel, B=B, H=H, S=S, Dh=Dh, D=D),
        out_shape=jax.ShapeDtypeStruct((B, D), A_x.dtype),
        in_specs=[any_spec] * 11,
        out_specs=pl.BlockSpec(memory_space=pltpu.VMEM),
        scratch_shapes=[
            pltpu.VMEM((NB, G, C, Dh), A_k_cache.dtype),
            pltpu.VMEM((NB, G, C, Dh), A_v_cache.dtype),
            vm(x2d), vm(c), vm(w_mod), vm(A_wq), vm(A_wo), vm(B_w_r),
            vm(wg_t), vm(wu_t), vm(B_w_down),
            pltpu.VMEM((B * H, Dh), jnp.float32),
            pltpu.VMEM((B * H, Dh), jnp.float32),
            pltpu.SemaphoreType.DMA((NB,)),
            pltpu.SemaphoreType.DMA((NB,)),
            pltpu.SemaphoreType.DMA((9,)),
        ],
        compiler_params=pltpu.CompilerParams(
            vmem_limit_bytes=100 * 1024 * 1024,
            disable_bounds_checks=DBC,
        ),
    )(x2d, A_k_cache, A_v_cache, A_wq, A_wo, B_w_r, wg_t, wu_t, B_w_down, c, w_mod).reshape(B, Sq, D)
```

```python
import functools

import jax
import jax.numpy as jnp
from jax import lax
import jax.experimental.pallas as pl
import jax.experimental.pallas.tpu as pltpu

NT = (((1,), (1,)), ((), ()))
G = 8
PIECES = tuple(int(t) for t in "64x64x192x64x128".split("x"))
C = sum(PIECES)
NB = 3
WDR = 2


def _layernorm(x, eps=1e-5):
    m = jnp.mean(x, axis=-1, keepdims=True)
    d = x - m
    v = jnp.mean(d * d, axis=-1, keepdims=True)
    return d / jnp.sqrt(v + eps)


def _kernel(x_hbm, k_hbm, v_hbm, wq_hbm, wo_hbm, wr_hbm, wg_hbm, wu_hbm, wd_hbm,
            c_hbm, wmod_hbm, out_ref,
            kbuf, vbuf, x_vm, c_vm, wmod_vm, wq_vm, wo_vm, wr_vm, wg_vm, wu_vm, wd_vm,
            q_scr, o_scr, ksem, vsem, wsem, dsem, *, B, H, S, Dh, D):
    f32, bf16 = jnp.float32, jnp.bfloat16
    NG = B * H // G
    NC = S // C
    N = NG * NC
    F = wd_hbm.shape[0]

    def whole(src, dst, sem):
        return pltpu.make_async_copy(src, dst, sem)

    def piece(src, dst, sem, rows, cols, t):
        ncb = src.shape[1] // cols
        r0 = pl.multiple_of((t // ncb) * rows, rows)
        c0 = pl.multiple_of((t % ncb) * cols, cols)
        idx = (pl.ds(r0, rows), pl.ds(c0, cols))
        return pltpu.make_async_copy(src.at[idx], dst.at[idx], sem)

    def streams(jobs, n):
        def body(t, carry):
            for pos, (src, dst, sem, rows, cols, base) in enumerate(jobs):
                piece(src, dst, sem, rows, cols, base + t).start(priority=pos % 2)
            return carry
        if n == 1:
            body(0, 0)
        elif n > 1:
            lax.fori_loop(0, n, body, 0)

    def spread(src, dst, sem, rows, cols, ns):
        n = (src.shape[0] // rows) * (src.shape[1] // cols)
        h = n // ns
        streams([(src, dst, sem, rows, cols, o * h) for o in range(ns)], h)
        streams([(src, dst, sem, rows, cols, t) for t in range(ns * h, n)], 1)

    def start_step(i, slot):
        grp = i // NC
        c = i % NC
        b = grp // (H // G)
        h0 = (grp % (H // G)) * G
        off = 0
        for p in PIECES:
            for g in range(G):
                src = (b, h0 + g, pl.ds(c * C + off, p))
                dst = (slot, g, pl.ds(off, p))
                pltpu.make_async_copy(k_hbm.at[src], kbuf.at[dst], ksem.at[slot]).start(priority=0)
                pltpu.make_async_copy(v_hbm.at[src], vbuf.at[dst], vsem.at[slot]).start(priority=1)
            off += p

    def wait_k(slot):
        whole(kbuf.at[slot], kbuf.at[slot], ksem.at[slot]).wait()

    def wait_v(slot):
        whole(vbuf.at[slot], vbuf.at[slot], vsem.at[slot]).wait()

    wd_blocks = [(a, min(a + 128, F)) for a in range(0, F, 128)]
    wd_rounds = [wd_blocks[r::WDR] for r in range(WDR)]

    def start_wd():
        for r, blocks in enumerate(wd_rounds):
            for t in range(4):
                jobs = [(wd_hbm, wd_vm, dsem.at[r], 32, D, a // 32 + t) for a, e in blocks if a + 32 * t < e]
                streams(jobs, 1)

    whole(c_hbm, c_vm, wsem.at[0]).start()
    whole(x_hbm, x_vm, wsem.at[1]).start(priority=1)
    spread(wmod_hbm, wmod_vm, wsem.at[2], 16, 1024, 4)
    spread(wq_hbm, wq_vm, wsem.at[3], 16, 1024, 4)
    for j in range(NB - 1):
        start_step(j, j)

    whole(c_hbm, c_vm, wsem.at[0]).wait()
    whole(wmod_hbm, wmod_vm, wsem.at[2]).wait()
    c = c_vm[...].astype(f32)
    sc = (c * jax.nn.sigmoid(c)).astype(bf16)
    mod = jnp.dot(sc, wmod_vm[...], preferred_element_type=f32)
    sa, ca, ga, sb, cb, gb = (mod[:, i * D:(i + 1) * D] for i in range(6))
    whole(x_hbm, x_vm, wsem.at[1]).wait()
    x = x_vm[...].astype(f32)
    h = (_layernorm(x) * (1.0 + ca) + sa).astype(bf16)
    whole(wq_hbm, wq_vm, wsem.at[3]).wait()
    q = jnp.dot(h, wq_vm[...], preferred_element_type=f32)
    for hh in range(H):
        q_scr[pl.ds(hh, B, stride=H), :] = q[:, hh * Dh:(hh + 1) * Dh]

    scale = float(Dh) ** -0.5
    row = lax.broadcasted_iota(jnp.int32, (G, Dh), 0)

    def group(grp, carry):
        qg = q_scr[pl.ds(pl.multiple_of(grp * G, G), G), :].astype(bf16)

        def step(c, carry):
            m_prev, l_prev, o_prev = carry
            i = grp * NC + c
            slot = i % NB

            @pl.when(i + NB - 1 < N)
            def _():
                start_step(i + NB - 1, (i + NB - 1) % NB)

            @pl.when(i + NB - 1 == N)
            def _():
                whole(wr_hbm, wr_vm, wsem.at[5]).start()
                spread(wo_hbm, wo_vm, wsem.at[4], 32, D, 4)

            @pl.when(i + NB - 2 == N)
            def _():
                spread(wg_hbm, wg_vm, wsem.at[6], 32, D, 2)
                spread(wu_hbm, wu_vm, wsem.at[7], 32, D, 2)
                start_wd()

            wait_k(slot)
            s = None
            for g in range(G):
                sg = lax.dot_general(qg, kbuf[slot, g], NT, preferred_element_type=f32)
                s = sg if s is None else jnp.where(row[:, :1] == g, sg, s)
            s = s * scale
            m_new = jnp.maximum(m_prev, jnp.max(s, axis=-1, keepdims=True))
            m_safe = jnp.where(m_new == -jnp.inf, 0.0, m_new)
            p = jnp.exp(s - m_safe)
            alpha = jnp.exp(m_prev - m_safe)
            l_new = alpha * l_prev + jnp.sum(p, axis=-1, keepdims=True)
            pb = p.astype(bf16)
            wait_v(slot)
            r = None
            for g in range(G):
                rg = jnp.dot(pb, vbuf[slot, g], preferred_element_type=f32)
                r = rg if r is None else jnp.where(row == g, rg, r)
            o_new = alpha * o_prev + r
            return m_new, l_new, o_new

        init = (jnp.full((G, 1), -jnp.inf, f32), jnp.zeros((G, 1), f32), jnp.zeros((G, Dh), f32))
        m, l, o = lax.fori_loop(0, NC, step, init)
        o_scr[pl.ds(pl.multiple_of(grp * G, G), G), :] = o / l
        return carry

    lax.fori_loop(0, NG, group, 0)

    o_all = jnp.concatenate(
        [o_scr[pl.ds(hh, B, stride=H), :] for hh in range(H)], axis=1).astype(bf16)
    whole(wo_hbm, wo_vm, wsem.at[4]).wait()
    attn = jnp.dot(o_all, wo_vm[...], preferred_element_type=f32)
    x2 = x + ga * attn
    h2 = _layernorm(x2) * (1.0 + cb) + sb
    h2b = h2.astype(bf16)
    whole(wr_hbm, wr_vm, wsem.at[5]).wait()
    r = jnp.sum(h2 * wr_vm[...].astype(f32).reshape(1, D), axis=-1, keepdims=True)
    whole(wg_hbm, wg_vm, wsem.at[6]).wait()
    g = lax.dot_general(h2b, wg_vm[...], NT, preferred_element_type=f32)
    g = g * jax.nn.sigmoid(g)
    whole(wu_hbm, wu_vm, wsem.at[7]).wait()
    u = lax.dot_general(h2b, wu_vm[...], NT, preferred_element_type=f32)
    gu = (g * u).astype(bf16)
    y = None
    for rr, blocks in enumerate(wd_rounds):
        for a, e in blocks:
            whole(wd_hbm.at[pl.ds(a, e - a)], wd_vm.at[pl.ds(a, e - a)], dsem.at[rr]).wait()
        for a, e in blocks:
            yn = jnp.dot(gu[:, a:e], wd_vm[pl.ds(a, e - a), :], preferred_element_type=f32)
            y = yn if y is None else y + yn
    y = y * jax.nn.sigmoid(r)
    upd = h2 * 0.0 + y
    out = x2 + gb * (h2 + upd)
    out_ref[...] = out.astype(out_ref.dtype)


@jax.jit
def pallas_adaLN_cond__gqa_block_cached__moe_arch_mod__decode_kernel(
    A_x: jax.Array,
    A_k_cache: jax.Array,
    A_v_cache: jax.Array,
    A_wq: jax.Array,
    A_wo: jax.Array,
    B_x: jax.Array,
    B_w_r: jax.Array,
    B_w_gate: jax.Array,
    B_w_up: jax.Array,
    B_w_down: jax.Array,
    c: jax.Array,
    w_mod: jax.Array,
):
    del B_x
    B, Sq, D = A_x.shape
    _, H, S, Dh = A_k_cache.shape
    assert Sq == 1 and A_wq.shape == (D, H * Dh)
    assert H % G == 0 and S % C == 0

    x2d = A_x.reshape(B, D)
    wg_t = B_w_gate.T
    wu_t = B_w_up.T

    def vm(a):
        return pltpu.VMEM(a.shape, a.dtype)

    any_spec = pl.BlockSpec(memory_space=pltpu.HBM)
    return pl.pallas_call(
        functools.partial(_kernel, B=B, H=H, S=S, Dh=Dh, D=D),
        out_shape=jax.ShapeDtypeStruct((B, D), A_x.dtype),
        in_specs=[any_spec] * 11,
        out_specs=pl.BlockSpec(memory_space=pltpu.VMEM),
        scratch_shapes=[
            pltpu.VMEM((NB, G, C, Dh), A_k_cache.dtype),
            pltpu.VMEM((NB, G, C, Dh), A_v_cache.dtype),
            vm(x2d), vm(c), vm(w_mod), vm(A_wq), vm(A_wo), vm(B_w_r),
            vm(wg_t), vm(wu_t), vm(B_w_down),
            pltpu.VMEM((B * H, Dh), jnp.float32),
            pltpu.VMEM((B * H, Dh), jnp.float32),
            pltpu.SemaphoreType.DMA((NB,)),
            pltpu.SemaphoreType.DMA((NB,)),
            pltpu.SemaphoreType.DMA((9,)),
            pltpu.SemaphoreType.DMA((WDR,)),
        ],
        compiler_params=pltpu.CompilerParams(
            vmem_limit_bytes=100 * 1024 * 1024,
            disable_bounds_checks=False,
        ),
    )(x2d, A_k_cache, A_v_cache, A_wq, A_wo, B_w_r, wg_t, wu_t, B_w_down, c, w_mod).reshape(B, Sq, D)
```

```python
import functools

import jax
import jax.numpy as jnp
from jax import lax
import jax.experimental.pallas as pl
import jax.experimental.pallas.tpu as pltpu

NT = (((1,), (1,)), ((), ()))
G = 8
PIECES = (64, 64, 128, 64, 64, 128)
C = sum(PIECES)
NB = 3
PIECE_BYTES = 32 * 1024


def _layernorm(x, eps=1e-5):
    m = jnp.mean(x, axis=-1, keepdims=True)
    d = x - m
    v = jnp.mean(d * d, axis=-1, keepdims=True)
    return d / jnp.sqrt(v + eps)


def _kernel(x_hbm, k_hbm, v_hbm, wq_hbm, wo_hbm, wr_hbm, wg_hbm, wu_hbm, wd_hbm,
            c_hbm, wmod_hbm, out_ref,
            kbuf, vbuf, x_vm, c_vm, wmod_vm, wq_vm, wo_vm, wr_vm, wg_vm, wu_vm, wd_vm,
            q_scr, o_scr, ksem, vsem, wsem, *, B, H, S, Dh, D):
    f32, bf16 = jnp.float32, jnp.bfloat16
    NG = B * H // G
    NC = S // C
    N = NG * NC

    small = {
        "c": (c_hbm, c_vm, wsem.at[0]), "x": (x_hbm, x_vm, wsem.at[1]),
        "wmod": (wmod_hbm, wmod_vm, wsem.at[2]), "wq": (wq_hbm, wq_vm, wsem.at[3]),
        "wo": (wo_hbm, wo_vm, wsem.at[4]), "wr": (wr_hbm, wr_vm, wsem.at[5]),
        "wg": (wg_hbm, wg_vm, wsem.at[6]), "wu": (wu_hbm, wu_vm, wsem.at[7]),
        "wd": (wd_hbm, wd_vm, wsem.at[8]),
    }

    def whole(name):
        return pltpu.make_async_copy(*small[name])

    def start_spread(name, ns):
        src, dst, sem = small[name]
        cols = min(src.shape[1], 1024)
        rows = PIECE_BYTES // (2 * cols)
        assert src.shape[0] % rows == 0 and src.shape[1] % cols == 0
        ncb = src.shape[1] // cols
        n = (src.shape[0] // rows) * ncb
        per = n // ns

        def start(t, thread):
            idx = (pl.ds(pl.multiple_of((t // ncb) * rows, rows), rows),
                   pl.ds(pl.multiple_of((t % ncb) * cols, cols), cols))
            pltpu.make_async_copy(src.at[idx], dst.at[idx], sem).start(priority=thread)

        def body(t, carry):
            for o in range(ns):
                start(o * per + t, o % 2)
            return carry

        lax.fori_loop(0, per, body, 0)
        for t in range(ns * per, n):
            start(t, t % 2)

    def start_step(i, slot):
        grp, c = i // NC, i % NC
        b, h0 = grp // (H // G), (grp % (H // G)) * G
        off = 0
        for p in PIECES:
            for g in range(G):
                src = (b, h0 + g, pl.ds(c * C + off, p))
                dst = (slot, g, pl.ds(off, p))
                pltpu.make_async_copy(k_hbm.at[src], kbuf.at[dst], ksem.at[slot]).start(priority=0)
                pltpu.make_async_copy(v_hbm.at[src], vbuf.at[dst], vsem.at[slot]).start(priority=1)
            off += p

    def wait_slot(buf, sem, slot):
        pltpu.make_async_copy(buf.at[slot], buf.at[slot], sem.at[slot]).wait()

    whole("c").start(priority=0)
    whole("x").start(priority=1)
    start_spread("wmod", 4)
    start_spread("wq", 4)
    for j in range(NB - 1):
        start_step(j, j)

    whole("c").wait()
    whole("wmod").wait()
    c = c_vm[...].astype(f32)
    sc = (c * jax.nn.sigmoid(c)).astype(bf16)
    mod = jnp.dot(sc, wmod_vm[...], preferred_element_type=f32)
    sa, ca, ga, sb, cb, gb = (mod[:, i * D:(i + 1) * D] for i in range(6))
    whole("x").wait()
    x = x_vm[...].astype(f32)
    h = (_layernorm(x) * (1.0 + ca) + sa).astype(bf16)
    whole("wq").wait()
    q = jnp.dot(h, wq_vm[...], preferred_element_type=f32)
    for hh in range(H):
        q_scr[pl.ds(hh, B, stride=H), :] = q[:, hh * Dh:(hh + 1) * Dh]

    scale = float(Dh) ** -0.5
    row = lax.broadcasted_iota(jnp.int32, (G, Dh), 0)

    def group(grp, carry):
        rows = pl.ds(pl.multiple_of(grp * G, G), G)
        qg = q_scr[rows, :].astype(bf16)

        def step(c, carry):
            m_prev, l_prev, o_prev = carry
            i = grp * NC + c
            slot = i % NB

            @pl.when(i + NB - 1 < N)
            def _():
                start_step(i + NB - 1, (i + NB - 1) % NB)

            @pl.when(i + NB - 1 == N)
            def _():
                whole("wr").start()
                start_spread("wo", 4)

            @pl.when(i + NB - 2 == N)
            def _():
                start_spread("wg", 2)
                start_spread("wu", 2)
                start_spread("wd", 2)

            wait_slot(kbuf, ksem, slot)
            s = None
            for g in range(G):
                sg = lax.dot_general(qg, kbuf[slot, g], NT, preferred_element_type=f32)
                s = sg if s is None else jnp.where(row[:, :1] == g, sg, s)
            s = s * scale
            m_new = jnp.maximum(m_prev, jnp.max(s, axis=-1, keepdims=True))
            m_safe = jnp.where(m_new == -jnp.inf, 0.0, m_new)
            p = jnp.exp(s - m_safe)
            alpha = jnp.exp(m_prev - m_safe)
            l_new = alpha * l_prev + jnp.sum(p, axis=-1, keepdims=True)
            pb = p.astype(bf16)
            wait_slot(vbuf, vsem, slot)
            r = None
            for g in range(G):
                rg = jnp.dot(pb, vbuf[slot, g], preferred_element_type=f32)
                r = rg if r is None else jnp.where(row == g, rg, r)
            return m_new, l_new, alpha * o_prev + r

        init = (jnp.full((G, 1), -jnp.inf, f32), jnp.zeros((G, 1), f32), jnp.zeros((G, Dh), f32))
        _, l, o = lax.fori_loop(0, NC, step, init)
        o_scr[rows, :] = o / l
        return carry

    lax.fori_loop(0, NG, group, 0)

    o_all = jnp.concatenate(
        [o_scr[pl.ds(hh, B, stride=H), :] for hh in range(H)], axis=1).astype(bf16)
    whole("wo").wait()
    attn = jnp.dot(o_all, wo_vm[...], preferred_element_type=f32)
    x2 = x + ga * attn
    h2 = _layernorm(x2) * (1.0 + cb) + sb
    h2b = h2.astype(bf16)

    whole("wr").wait()
    r = jnp.sum(h2 * wr_vm[...].astype(f32).reshape(1, D), axis=-1, keepdims=True)
    whole("wg").wait()
    g = lax.dot_general(h2b, wg_vm[...], NT, preferred_element_type=f32)
    g = g * jax.nn.sigmoid(g)
    whole("wu").wait()
    u = lax.dot_general(h2b, wu_vm[...], NT, preferred_element_type=f32)
    gu = (g * u).astype(bf16)
    whole("wd").wait()
    y = jnp.dot(gu, wd_vm[...], preferred_element_type=f32)
    y = y * jax.nn.sigmoid(r)
    upd = h2 * 0.0 + y
    out_ref[...] = (x2 + gb * (h2 + upd)).astype(out_ref.dtype)


@jax.jit
def pallas_adaLN_cond__gqa_block_cached__moe_arch_mod__decode_kernel(
    A_x: jax.Array,
    A_k_cache: jax.Array,
    A_v_cache: jax.Array,
    A_wq: jax.Array,
    A_wo: jax.Array,
    B_x: jax.Array,
    B_w_r: jax.Array,
    B_w_gate: jax.Array,
    B_w_up: jax.Array,
    B_w_down: jax.Array,
    c: jax.Array,
    w_mod: jax.Array,
):
    del B_x
    B, Sq, D = A_x.shape
    _, H, S, Dh = A_k_cache.shape
    assert Sq == 1 and A_wq.shape == (D, H * Dh) and A_v_cache.shape == A_k_cache.shape
    assert H % G == 0 and S % C == 0

    x2d = A_x.reshape(B, D)
    wg_t = B_w_gate.T
    wu_t = B_w_up.T

    def vmem_like(a):
        return pltpu.VMEM(a.shape, a.dtype)

    out = pl.pallas_call(
        functools.partial(_kernel, B=B, H=H, S=S, Dh=Dh, D=D),
        out_shape=jax.ShapeDtypeStruct((B, D), A_x.dtype),
        in_specs=[pl.BlockSpec(memory_space=pltpu.HBM)] * 11,
        out_specs=pl.BlockSpec(memory_space=pltpu.VMEM),
        scratch_shapes=[
            pltpu.VMEM((NB, G, C, Dh), A_k_cache.dtype),
            pltpu.VMEM((NB, G, C, Dh), A_v_cache.dtype),
            vmem_like(x2d), vmem_like(c), vmem_like(w_mod), vmem_like(A_wq), vmem_like(A_wo),
            vmem_like(B_w_r), vmem_like(wg_t), vmem_like(wu_t), vmem_like(B_w_down),
            pltpu.VMEM((B * H, Dh), jnp.float32),
            pltpu.VMEM((B * H, Dh), jnp.float32),
            pltpu.SemaphoreType.DMA((NB,)),
            pltpu.SemaphoreType.DMA((NB,)),
            pltpu.SemaphoreType.DMA((9,)),
        ],
        compiler_params=pltpu.CompilerParams(vmem_limit_bytes=64 * 1024 * 1024),
    )(x2d, A_k_cache, A_v_cache, A_wq, A_wo, B_w_r, wg_t, wu_t, B_w_down, c, w_mod)
    return out.reshape(B, Sq, D)
```

```python
import functools

import jax
import jax.numpy as jnp
from jax import lax
import jax.experimental.pallas as pl
import jax.experimental.pallas.tpu as pltpu

NT = (((1,), (1,)), ((), ()))
G = 8
K_PIECES = (64, 64, 192, 64, 128)
V_PIECES = (64, 64, 128, 64, 64, 128)
C = sum(K_PIECES)
assert sum(V_PIECES) == C
NB = 3
PIECE_BYTES = 32 * 1024


def _layernorm(x, eps=1e-5):
    m = jnp.mean(x, axis=-1, keepdims=True)
    d = x - m
    v = jnp.mean(d * d, axis=-1, keepdims=True)
    return d / jnp.sqrt(v + eps)


def _kernel(x_hbm, k_hbm, v_hbm, wq_hbm, wo_hbm, wr_hbm, wg_hbm, wu_hbm, wd_hbm,
            c_hbm, wmod_hbm, out_ref,
            kbuf, vbuf, x_vm, c_vm, wmod_vm, wq_vm, wo_vm, wr_vm, wg_vm, wu_vm, wd_vm,
            q_scr, o_scr, ksem, vsem, wsem, *, B, H, S, Dh, D):
    f32, bf16 = jnp.float32, jnp.bfloat16
    NG = B * H // G
    NC = S // C
    N = NG * NC

    small = {
        "c": (c_hbm, c_vm, wsem.at[0]), "x": (x_hbm, x_vm, wsem.at[1]),
        "wmod": (wmod_hbm, wmod_vm, wsem.at[2]), "wq": (wq_hbm, wq_vm, wsem.at[3]),
        "wo": (wo_hbm, wo_vm, wsem.at[4]), "wr": (wr_hbm, wr_vm, wsem.at[5]),
        "wg": (wg_hbm, wg_vm, wsem.at[6]), "wu": (wu_hbm, wu_vm, wsem.at[7]),
        "wd": (wd_hbm, wd_vm, wsem.at[8]),
    }

    def whole(name):
        return pltpu.make_async_copy(*small[name])

    def start_spread(name, ns):
        src, dst, sem = small[name]
        cols = min(src.shape[1], 1024)
        rows = PIECE_BYTES // (2 * cols)
        assert src.shape[0] % rows == 0 and src.shape[1] % cols == 0
        ncb = src.shape[1] // cols
        n = (src.shape[0] // rows) * ncb
        per = n // ns

        def start(t, thread):
            idx = (pl.ds(pl.multiple_of((t // ncb) * rows, rows), rows),
                   pl.ds(pl.multiple_of((t % ncb) * cols, cols), cols))
            pltpu.make_async_copy(src.at[idx], dst.at[idx], sem).start(priority=thread)

        def body(t, carry):
            for o in range(ns):
                start(o * per + t, o % 2)
            return carry

        lax.fori_loop(0, per, body, 0)
        for t in range(ns * per, n):
            start(t, t % 2)

    def start_step(i, slot):
        grp, c = i // NC, i % NC
        b, h0 = grp // (H // G), (grp % (H // G)) * G
        for j in range(max(len(K_PIECES), len(V_PIECES))):
            for g in range(G):
                for thread, (pieces, hbm, buf, sem) in enumerate(
                        ((K_PIECES, k_hbm, kbuf, ksem), (V_PIECES, v_hbm, vbuf, vsem))):
                    if j < len(pieces):
                        off, n = sum(pieces[:j]), pieces[j]
                        pltpu.make_async_copy(
                            hbm.at[b, h0 + g, pl.ds(c * C + off, n)],
                            buf.at[slot, g, pl.ds(off, n)],
                            sem.at[slot]).start(priority=thread)

    def wait_slot(buf, sem, slot):
        pltpu.make_async_copy(buf.at[slot], buf.at[slot], sem.at[slot]).wait()

    whole("c").start(priority=0)
    whole("x").start(priority=1)
    start_spread("wmod", 4)
    start_spread("wq", 4)
    for j in range(NB - 1):
        start_step(j, j)

    whole("c").wait()
    whole("wmod").wait()
    c = c_vm[...].astype(f32)
    sc = (c * jax.nn.sigmoid(c)).astype(bf16)
    mod = jnp.dot(sc, wmod_vm[...], preferred_element_type=f32)
    sa, ca, ga, sb, cb, gb = (mod[:, i * D:(i + 1) * D] for i in range(6))
    whole("x").wait()
    x = x_vm[...].astype(f32)
    h = (_layernorm(x) * (1.0 + ca) + sa).astype(bf16)
    whole("wq").wait()
    q = jnp.dot(h, wq_vm[...], preferred_element_type=f32)
    for hh in range(H):
        q_scr[pl.ds(hh, B, stride=H), :] = q[:, hh * Dh:(hh + 1) * Dh]

    scale = float(Dh) ** -0.5
    row = lax.broadcasted_iota(jnp.int32, (G, Dh), 0)

    def group(grp, carry):
        rows = pl.ds(pl.multiple_of(grp * G, G), G)
        qg = q_scr[rows, :].astype(bf16)

        def step(c, carry):
            m_prev, l_prev, o_prev = carry
            i = grp * NC + c
            slot = i % NB

            @pl.when(i + NB - 1 < N)
            def _():
                start_step(i + NB - 1, (i + NB - 1) % NB)

            @pl.when(i + NB - 1 == N)
            def _():
                whole("wr").start()
                start_spread("wo", 4)

            @pl.when(i + NB - 2 == N)
            def _():
                start_spread("wg", 2)
                start_spread("wu", 2)
                start_spread("wd", 2)

            wait_slot(kbuf, ksem, slot)
            s = None
            for g in range(G):
                sg = lax.dot_general(qg, kbuf[slot, g], NT, preferred_element_type=f32)
                s = sg if s is None else jnp.where(row[:, :1] == g, sg, s)
            s = s * scale
            m_new = jnp.maximum(m_prev, jnp.max(s, axis=-1, keepdims=True))
            m_safe = jnp.where(m_new == -jnp.inf, 0.0, m_new)
            p = jnp.exp(s - m_safe)
            alpha = jnp.exp(m_prev - m_safe)
            l_new = alpha * l_prev + jnp.sum(p, axis=-1, keepdims=True)
            pb = p.astype(bf16)
            wait_slot(vbuf, vsem, slot)
            r = None
            for g in range(G):
                rg = jnp.dot(pb, vbuf[slot, g], preferred_element_type=f32)
                r = rg if r is None else jnp.where(row == g, rg, r)
            return m_new, l_new, alpha * o_prev + r

        init = (jnp.full((G, 1), -jnp.inf, f32), jnp.zeros((G, 1), f32), jnp.zeros((G, Dh), f32))
        _, l, o = lax.fori_loop(0, NC, step, init)
        o_scr[rows, :] = o / l
        return carry

    lax.fori_loop(0, NG, group, 0)

    o_all = jnp.concatenate(
        [o_scr[pl.ds(hh, B, stride=H), :] for hh in range(H)], axis=1).astype(bf16)
    whole("wo").wait()
    attn = jnp.dot(o_all, wo_vm[...], preferred_element_type=f32)
    x2 = x + ga * attn
    h2 = _layernorm(x2) * (1.0 + cb) + sb
    h2b = h2.astype(bf16)

    whole("wr").wait()
    r = jnp.sum(h2 * wr_vm[...].astype(f32).reshape(1, D), axis=-1, keepdims=True)
    whole("wg").wait()
    g = lax.dot_general(h2b, wg_vm[...], NT, preferred_element_type=f32)
    g = g * jax.nn.sigmoid(g)
    whole("wu").wait()
    u = lax.dot_general(h2b, wu_vm[...], NT, preferred_element_type=f32)
    gu = (g * u).astype(bf16)
    whole("wd").wait()
    y = jnp.dot(gu, wd_vm[...], preferred_element_type=f32)
    y = y * jax.nn.sigmoid(r)
    upd = h2 * 0.0 + y
    out_ref[...] = (x2 + gb * (h2 + upd)).astype(out_ref.dtype)


@jax.jit
def pallas_adaLN_cond__gqa_block_cached__moe_arch_mod__decode_kernel(
    A_x: jax.Array,
    A_k_cache: jax.Array,
    A_v_cache: jax.Array,
    A_wq: jax.Array,
    A_wo: jax.Array,
    B_x: jax.Array,
    B_w_r: jax.Array,
    B_w_gate: jax.Array,
    B_w_up: jax.Array,
    B_w_down: jax.Array,
    c: jax.Array,
    w_mod: jax.Array,
):
    del B_x
    B, Sq, D = A_x.shape
    _, H, S, Dh = A_k_cache.shape
    assert Sq == 1 and A_wq.shape == (D, H * Dh) and A_v_cache.shape == A_k_cache.shape
    assert H % G == 0 and S % C == 0

    x2d = A_x.reshape(B, D)
    wg_t = B_w_gate.T
    wu_t = B_w_up.T

    def vmem_like(a):
        return pltpu.VMEM(a.shape, a.dtype)

    out = pl.pallas_call(
        functools.partial(_kernel, B=B, H=H, S=S, Dh=Dh, D=D),
        out_shape=jax.ShapeDtypeStruct((B, D), A_x.dtype),
        in_specs=[pl.BlockSpec(memory_space=pltpu.HBM)] * 11,
        out_specs=pl.BlockSpec(memory_space=pltpu.VMEM),
        scratch_shapes=[
            pltpu.VMEM((NB, G, C, Dh), A_k_cache.dtype),
            pltpu.VMEM((NB, G, C, Dh), A_v_cache.dtype),
            vmem_like(x2d), vmem_like(c), vmem_like(w_mod), vmem_like(A_wq), vmem_like(A_wo),
            vmem_like(B_w_r), vmem_like(wg_t), vmem_like(wu_t), vmem_like(B_w_down),
            pltpu.VMEM((B * H, Dh), jnp.float32),
            pltpu.VMEM((B * H, Dh), jnp.float32),
            pltpu.SemaphoreType.DMA((NB,)),
            pltpu.SemaphoreType.DMA((NB,)),
            pltpu.SemaphoreType.DMA((9,)),
        ],
        compiler_params=pltpu.CompilerParams(vmem_limit_bytes=64 * 1024 * 1024),
    )(x2d, A_k_cache, A_v_cache, A_wq, A_wo, B_w_r, wg_t, wu_t, B_w_down, c, w_mod)
    return out.reshape(B, Sq, D)
```
